```python
import os as _os
_os.environ.setdefault("JAX_PLATFORMS", "cpu")
import jax
import jax.numpy as jnp

def _softmax(x, axis=-1):
    return jax.nn.softmax(x, axis=axis)
def _gelu(x):
    return jax.nn.gelu(x, approximate=True)
def _silu(x):
    return jax.nn.silu(x)
def _sigmoid(x):
    return jax.nn.sigmoid(x)
def _layernorm(x, axis=-1, eps=1e-5):
    m = jnp.mean(x, axis=axis, keepdims=True)
    v = jnp.var(x, axis=axis, keepdims=True)
    return (x - m) / jnp.sqrt(v + eps)
def _scatter_add(tgt, idx, src, axis=0):
    return tgt.at[idx].add(src)
def _segment_sum(src, seg, n):
    return jax.ops.segment_sum(src, seg, n)
class _Rng:
    def __init__(self, key):
        self._k = key
    def _next(self):
        self._k, sub = jax.random.split(self._k)
        return sub
    def normal(self, shape):
        return jax.random.normal(self._next(), shape, dtype=jnp.bfloat16)
    def randint(self, lo, hi, shape):
        return jax.random.randint(self._next(), shape, lo, hi, dtype=jnp.int32)
    def uniform(self, shape, lo=0.0, hi=1.0):
        return jax.random.uniform(self._next(), shape, jnp.bfloat16, lo, hi)
    def permutation(self, n):
        return jax.random.permutation(self._next(), n)


kernel_name = 'concat_heads__ssm_conv_h3__sliding_block__prompt'

def setup_inputs():
    _rng = _Rng(jax.random.key(int.from_bytes(__import__("os").urandom(4), "little")))
    _w = (lambda a: (lambda t: t.astype(jnp.bfloat16) if jnp.issubdtype(t.dtype, jnp.floating) else t)(jnp.asarray(a)))
    def _A_setup():
        B, S, D = 1, 2048, 512
        ks = 4
        return {
            "q": _w((lambda *s: _rng.normal(s) * 0.05)(B, S, D)),
            "k": _w((lambda *s: _rng.normal(s) * 0.2)(B, S, D)),
            "v": _w((lambda *s: _rng.normal(s) * 0.2)(B, S, D)),
            "shift_k": _w((lambda *s: _rng.normal(s) * 0.2)(D, ks) * 0.5),
            "ssm_k": _w((lambda *s: _rng.normal(s) * 0.2)(D, S) * (1.0 / S ** 0.5)),
            "ssm_D": _w((lambda *s: _rng.normal(s) * 0.2)(D)),
        }
    _A_in = _A_setup()

    def _B_setup():
        B, S, D = 1, 2048, 512
        return {
            "x": _w((lambda *s: _rng.normal(s) * 0.2)(B, S, D)),
            "wqkv": _w((lambda *s: _rng.normal(s) * 0.2)(D, 3 * D)),
            "wo": _w((lambda *s: _rng.normal(s) * 0.05)(D, D)),
        }
    _B_in = _B_setup()

    return {
        "A_q": _A_in["q"],
        "A_k": _A_in["k"],
        "A_v": _A_in["v"],
        "A_shift_k": _A_in["shift_k"],
        "A_ssm_k": _A_in["ssm_k"],
        "A_ssm_D": _A_in["ssm_D"],
        "B_x": _B_in["x"],
        "B_wqkv": _B_in["wqkv"],
        "B_wo": _B_in["wo"],
    }

def reference(A_q, A_k, A_v, A_shift_k, A_ssm_k, A_ssm_D, B_x, B_wqkv, B_wo):
    def _A_ref(q, k, v, shift_k, ssm_k, ssm_D):
        B, S, D = q.shape
        ks = shift_k.shape[-1]
        k_pad = jnp.pad(k, ((0, 0), (ks - 1, 0), (0, 0)))
        k_shift = jnp.zeros_like(k)
        for t in range(ks):
            k_shift = k_shift + k_pad[:, t:t + S, :] * shift_k[:, ks - 1 - t][None, None, :]
        kv = k_shift * v
        L = 2 * S
        kv_pad = jnp.pad(kv, ((0, 0), (0, S), (0, 0)))
        kf_pad = jnp.pad(ssm_k, ((0, 0), (0, S)))
        kv_f = (lambda x, axes=(-2,-1): jnp.fft.rfft2(x.astype(jnp.float32), axes=axes))(kv_pad[:, None, :, :], axes=(1, 2))
        kf_f = (lambda x, axes=(-2,-1): jnp.fft.rfft2(x.astype(jnp.float32), axes=axes))(kf_pad[:, None, :], axes=(1, 2))
        kf_f = (lambda x, *d: x.transpose(*d))(kf_f, 1, 2, 0)
        y_f = kv_f * kf_f[None, :, :, :]
        y = (lambda x, s, axes=(-2,-1): jnp.fft.irfft2(x, s=s, axes=axes).astype(jnp.bfloat16))(y_f, (1, L), axes=(1, 2))[:, 0, :S, :]
        y = y + kv * ssm_D[None, None, :]
        return q * y

    def _B_ref(x, wqkv, wo):
        B, S, D = x.shape
        H = 32; Dh = D // H; W = 256
        qkv = (lambda x, *d: x.transpose(*d))((x @ wqkv).reshape(B, S, 3, H, Dh), 2, 0, 3, 1, 4)
        q, k, v = qkv[0], qkv[1], qkv[2]
        scores = jnp.einsum("bhqd,bhkd->bhqk", q, k) * (Dh ** -0.5)
        idx = jnp.arange(S)
        mask = (idx[:, None] - idx[None, :] >= 0) & (idx[:, None] - idx[None, :] < W)
        scores = jnp.where(mask[None, None], scores, -1e9)
        p = _softmax(scores, axis=-1)
        o = jnp.einsum("bhqk,bhkd->bhqd", p, v)
        return (lambda x, *d: x.transpose(*d))(o, 0, 2, 1, 3).reshape(B, S, D) @ wo

    a = _A_ref(A_q, A_k, A_v, A_shift_k, A_ssm_k, A_ssm_D)
    b = _B_ref(B_x, B_wqkv, B_wo)
    return jnp.concatenate([a, b], axis=-1)
```

```python
import numpy as np
import ml_dtypes
import jax
import jax.numpy as jnp
import jax.experimental.pallas as pl
import jax.experimental.pallas.tpu as pltpu

S, D, C = 2048, 512, 128
NC = S // C
NG = D // 128
F32, BF = jnp.float32, jnp.bfloat16
NT = (((1,), (1,)), ((), ()))
TN = (((0,), (0,)), ((), ()))

_k = np.arange(C)[:, None] + 0.5
_t = np.arange(C)[None, :]
_ang = 2.0 * np.pi * _k * _t / (2 * C)
_FWD = np.concatenate([np.cos(_ang), -np.sin(_ang)], 0).astype(ml_dtypes.bfloat16)
_INV = (np.concatenate([np.cos(_ang).T, -np.sin(_ang).T], 1) / C).astype(ml_dtypes.bfloat16)


def _dot(a, b, dims=(((1,), (0,)), ((), ()))):
    return jax.lax.dot_general(a, b, dims, preferred_element_type=F32)


def _kernel(q_h, k_h, v_h, sk_ref, h_h, d_ref, x_h, w_h, wo_h, f_ref, g_ref, o_h,
            xb, wb, wT, wob, qT, kb, vT, aq, ak, av, hb, kvb, X, H, Z, oT, ob, W, Sb, sem, osem):
    cp = pltpu.make_async_copy
    XC = 512
    c_w = cp(w_h, wb, sem.at[0])
    c_x = [cp(x_h.at[pl.ds(i * XC, XC)], xb.at[pl.ds(i * XC, XC)], sem.at[1 + i]) for i in range(4)]
    c_k = cp(k_h, ak.at[pl.ds(16, S)], sem.at[5])
    c_v = cp(v_h, av, sem.at[6])
    c_h = cp(h_h, hb, sem.at[7])
    c_o = cp(wo_h, wob, sem.at[8])
    c_q = cp(q_h, aq, sem.at[9])
    for c in [c_w] + c_x + [c_k, c_v, c_h, c_o, c_q]:
        c.start()
    ak[0:16, :] = jnp.zeros((16, D), BF)
    for g in range(NG):
        kb[g, 0:256, :] = jnp.zeros((256, 128), BF)
    vT[:, 0:16, 0:256] = jnp.zeros((32, 16, 256), BF)
    vT[:, 16:32, :] = jnp.ones((32, 16, S + 256), BF)
    W[...] = jnp.zeros((128, 8 * C), BF)

    c_w.wait()
    wT[0:D, :] = wb[:, 0:D].T
    wT[D:2 * D, :] = wb[:, 2 * D:3 * D].T
    qs = np.float32(0.25 * np.log2(np.e))
    for i in range(4):
        c_x[i].wait()
        xx = xb[pl.ds(i * XC, XC), :]
        qq = _dot(wT[0:D, :], xx, NT) * qs
        vv = _dot(wT[D:2 * D, :], xx, NT)
        kk = _dot(xx, wb[:, D:2 * D]).astype(BF)
        for b in range(4):
            qT[4 * i + b] = qq[:, b * 128:(b + 1) * 128].astype(BF)
        for h in range(32):
            vT[h, 0:16, pl.ds(256 + i * XC, XC)] = vv[16 * h:16 * h + 16].astype(BF)
        for g in range(NG):
            kb[g, pl.ds(256 + i * XC, XC), :] = kk[:, g * 128:(g + 1) * 128]

    eye = (jax.lax.broadcasted_iota(jnp.int32, (8, 4), 0)
           == jax.lax.broadcasted_iota(jnp.int32, (8, 4), 1)).astype(BF)
    taps = _dot(eye, sk_ref[...], NT)
    sgn = (1 - 2 * (jax.lax.broadcasted_iota(jnp.int32, (C, D), 0) % 2)).astype(F32)
    c_k.wait()
    c_v.wait()
    c_h.wait()

    prev = (jnp.zeros((C, D), F32), jnp.zeros((C, D), F32))
    for a in range(NC):
        prev = _fwd_static(a, prev, ak, av, kvb, taps, sgn, f_ref, hb, X, H)

    c_o.wait()
    upper = (jax.lax.broadcasted_iota(jnp.int32, (C, 4 * C), 0)
             > jax.lax.broadcasted_iota(jnp.int32, (C, 4 * C), 1) % C)
    ones = jnp.ones((16, 3 * C), BF)
    NEG = np.float32(-1e30)

    def mac(fb, g):
        rs = pl.ds(pl.multiple_of(fb * 8, 8), 8)
        ls = pl.ds(pl.multiple_of(g * 128, 128), 128)
        xs = {}
        for a0 in range(0, NC, 4):
            acc = [[None] * 3 for _ in range(4)]
            for j in range(a0 + 4):
                h0, h1, h2 = H[0, j, rs, ls], H[1, j, rs, ls], H[2, j, rs, ls]
                for u in range(4):
                    n = a0 + u - j
                    if n < 0:
                        continue
                    if n not in xs:
                        xs[n] = (X[0, n, rs, ls], X[1, n, rs, ls], X[2, n, rs, ls])
                    x0, x1, x2 = xs[n]
                    for w, t in enumerate((h0 * x2, x0 * h1, x1 * h2)):
                        acc[u][w] = t if acc[u][w] is None else acc[u][w] + t
            for u in range(4):
                Z[a0 + u, rs, ls] = acc[u][0] - acc[u][2]
                Z[a0 + u, pl.ds(pl.multiple_of(C + fb * 8, 8), 8), ls] = acc[u][0] + acc[u][1]

    def attn(qb, g, first):
        r0 = pl.multiple_of(qb * C, C)
        kt = kb[g, pl.ds(r0, 3 * C), :]
        for h in range(8):
            f0 = pl.multiple_of(g * 128 + h * 16, 16)
            W[16 * h:16 * h + 16, h * C:(h + 1) * C] = qT[qb, pl.ds(f0, 16), :]
        HW = 4 * C
        for hh in range(2):
            cs = slice(hh * HW, (hh + 1) * HW)
            s = _dot(kt, W[:, cs])
            s0, s1, s2 = s[:C], s[C:2 * C], s[2 * C:]
            if first <= 1:
                s0 = jnp.full((C, HW), NEG, F32)
            if first == 0:
                s1 = jnp.full((C, HW), NEG, F32)
            Sb[0, :, cs] = jnp.where(upper, s0, s2)
            Sb[1, :, cs] = s1
        for hh in range(2):
            os_ = []
            for h in range(4 * hh, 4 * hh + 4):
                cs = slice(h * C, (h + 1) * C)
                sc, s1 = Sb[0, :, cs], Sb[1, :, cs]
                m = jnp.max(jnp.maximum(sc, s1), axis=0, keepdims=True)
                pc = jnp.exp2(sc - m)
                p1 = jnp.exp2(s1 - m).astype(BF)
                p0 = jnp.where(upper[:, :C], pc, 0.0)
                vh = vT.at[g * 8 + h]
                os_.append(_dot(vh[:, pl.ds(r0, C)], p0.astype(BF))
                           + _dot(vh[:, pl.ds(r0 + C, C)], p1)
                           + _dot(vh[:, pl.ds(r0 + 2 * C, C)], (pc - p0).astype(BF)))
            for u, o in enumerate(os_):
                f0 = pl.multiple_of(g * 128 + (4 * hh + u) * 16, 16)
                oT[pl.ds(f0, 16), :] = (o[:16] / o[16:]).astype(BF)

    def block(qb, first):
        def body(g, c):
            attn(qb, g, first)
            mac(qb, g)
            return c
        jax.lax.fori_loop(0, NG, body, 0, unroll=4)
        r0 = pl.multiple_of(qb * C, C)
        ob[1, pl.ds(r0, C), :] = _dot(oT[...], wob[...], TN).astype(BF)

    block(0, 0)
    block(1, 1)
    jax.lax.fori_loop(2, NC, lambda qb, c: (block(qb, 2), c)[1], 0)
    c_b = cp(ob.at[1], o_h.at[:, pl.ds(D, D)], osem.at[0])
    c_b.start()

    c_q.wait()
    dd = d_ref[...].astype(F32)
    HS = S // 2
    c_a = [cp(ob.at[0, pl.ds(i * HS, HS)], o_h.at[pl.ds(i * HS, HS), pl.ds(0, D)], osem.at[1 + i])
           for i in range(2)]
    for a in range(NC):
        rs = pl.ds(a * C, C)
        y = _dot(g_ref[...], Z[a].astype(BF)).astype(BF).astype(F32)
        y = y + kvb[rs, :].astype(F32) * dd
        ob[0, rs, :] = (aq[rs, :].astype(F32) * y).astype(BF)
        if a == NC // 2 - 1:
            c_a[0].start()
    c_a[1].start()
    c_b.wait()
    c_a[0].wait()
    c_a[1].wait()


def _fwd_static(a, prev, ak, av, kvb, taps, sgn, f_ref, hb, X, H):
    r0 = a * C
    kf = ak[pl.ds(r0, C + 16), :].astype(F32)
    ks = kf[16:] * taps[0:1]
    for i in range(1, 4):
        ks = ks + kf[16 - i:16 - i + C] * taps[i:i + 1]
    kv = (ks * av[pl.ds(r0, C), :].astype(F32)).astype(BF)
    kvb[pl.ds(r0, C), :] = kv
    xf = _dot(f_ref[...], kv)
    xr, xi = xf[:C], xf[C:]
    X[0, a] = xr
    X[1, a] = xi
    X[2, a] = xr + xi
    hf = _dot(f_ref[...], hb[:, r0:r0 + C], NT)
    pr, pi = prev
    hr = hf[:C] - sgn * pi
    hi = hf[C:] + sgn * pr
    H[0, a] = hr
    H[1, a] = hi - hr
    H[2, a] = hr + hi
    return hf[:C], hf[C:]


@jax.jit
def pallas_concat_heads__ssm_conv_h3__sliding_block__prompt_kernel(
    A_q, A_k, A_v, A_shift_k, A_ssm_k, A_ssm_D, B_x, B_wqkv, B_wo):
    hbm = pl.BlockSpec(memory_space=pl.ANY)
    vm = pl.BlockSpec(memory_space=pltpu.VMEM)
    V = pltpu.VMEM
    sd = lambda: V((S, D), BF)
    out = pl.pallas_call(
        _kernel,
        out_shape=jax.ShapeDtypeStruct((S, 2 * D), BF),
        in_specs=[hbm, hbm, hbm, vm, hbm, vm, hbm, hbm, hbm, vm, vm],
        out_specs=hbm,
        scratch_shapes=[
            sd(), V((D, 3 * D), BF), V((2 * D, D), BF), V((D, D), BF),
            V((NC, D, C), BF), V((NG, S + 256, 128), BF), V((32, 32, S + 256), BF),
            sd(), V((S + 16, D), BF), sd(), V((D, S), BF), sd(),
            V((3, NC, C, D), F32), V((3, NC, C, D), F32), V((NC, 2 * C, D), F32),
            V((D, C), BF), V((2, S, D), BF), V((128, 8 * C), BF), V((2, C, 8 * C), F32),
            pltpu.SemaphoreType.DMA((10,)), pltpu.SemaphoreType.DMA((3,)),
        ],
        compiler_params=pltpu.CompilerParams(vmem_limit_bytes=100 * 1024 * 1024),
    )(A_q[0], A_k[0], A_v[0], A_shift_k, A_ssm_k, A_ssm_D.reshape(1, D), B_x[0], B_wqkv, B_wo,
      _FWD, _INV)
    return out[None]
```
